```python
import jax
import jax.numpy as jnp

def _softmax(x, axis=-1):
    return jax.nn.softmax(x, axis=axis)
def _gelu(x):
    return jax.nn.gelu(x, approximate=True)
def _silu(x):
    return jax.nn.silu(x)
def _sigmoid(x):
    return jax.nn.sigmoid(x)
def _layernorm(x, axis=-1, eps=1e-5):
    m = jnp.mean(x, axis=axis, keepdims=True)
    v = jnp.var(x, axis=axis, keepdims=True)
    return (x - m) / jnp.sqrt(v + eps)
def _scatter_add(tgt, idx, src, axis=0):
    return tgt.at[idx].add(src)
def _segment_sum(src, seg, n):
    return jax.ops.segment_sum(src, seg, n)
class _Rng:
    def __init__(self, key):
        self._k = key
    def _next(self):
        self._k, sub = jax.random.split(self._k)
        return sub
    def normal(self, shape):
        return jax.random.normal(self._next(), shape, dtype=jnp.bfloat16)
    def randint(self, lo, hi, shape):
        return jax.random.randint(self._next(), shape, lo, hi, dtype=jnp.int32)
    def uniform(self, shape, lo=0.0, hi=1.0):
        return jax.random.uniform(self._next(), shape, jnp.bfloat16, lo, hi)
    def permutation(self, n):
        return jax.random.permutation(self._next(), n)


kernel_name = 'standalone__modern_conv_block_slak__vision'

def setup_inputs():
    _rng = _Rng(jax.random.key(int.from_bytes(__import__("os").urandom(4), "little")))
    _w = (lambda a: (lambda t: t.astype(jnp.bfloat16) if jnp.issubdtype(t.dtype, jnp.floating) else t)(jnp.asarray(a)))
    H = W = 384
    C = 384
    K = 1
    return {
        "x": _w((lambda *s: _rng.normal(s) * 0.05)(1, H, W, C)),
        "dw": _w((lambda *s: _rng.normal(s) * 0.05)(K, K, C)),
        "w1": _w((lambda *s: _rng.normal(s) * 0.05)(C, 4 * C)),
        "w2": _w((lambda *s: _rng.normal(s) * 0.05)(4 * C, C)),
        "grn_g": _w((lambda *s: _rng.normal(s) * 0.05)(4 * C)),
        "grn_b": _w((lambda *s: _rng.normal(s) * 0.05)(4 * C)),
    }

def reference(x, dw, w1, w2, grn_g, grn_b):
    B, H, W, C = x.shape
    K = dw.shape[0]
    pad = K // 2
    xp = jnp.pad(x, ((0,0),(pad,pad),(pad,pad),(0,0)))
    out = jnp.zeros_like(x)
    for i in range(K):
        for j in range(K):
            out = out + xp[:, i:i+H, j:j+W, :] * dw[i, j][None, None, None, :]
    h = _layernorm(out, axis=-1)
    h = _gelu(h @ w1)
    gx = jnp.sqrt((h * h).sum(axis=(1, 2), keepdims=True) + 1e-6)
    nx = gx / (gx.mean(axis=-1, keepdims=True) + 1e-6)
    h = grn_g[None, None, None, :] * (h * nx) + grn_b[None, None, None, :] + h
    return x + h @ w2
```

```python
import functools
import jax, jax.numpy as jnp
from jax.experimental import pallas as pl
from jax.experimental.pallas import tpu as pltpu

C_TANH = 0.7978845608028654
C_CUBE = 0.044715
KS = (C_TANH * C_CUBE) ** (1.0 / 3.0)
A_LIN = C_TANH / KS
H_SCALE = 0.5 / KS


def make(TM=1024, SUB=512, NCH=1536, vmem=100):
    def kernel(x_ref, dw_ref, w1_ref, w2_ref, g_ref, b_ref, o_ref, h_hbm,
               hbuf, ssq_ref, w2s_ref, bias_ref, wsem, rsem):
        p = pl.program_id(0)
        i = pl.program_id(1)
        n = pl.num_programs(1)
        slot = i % 2

        def wcopy(t, s):
            return pltpu.make_async_copy(hbuf.at[s], h_hbm.at[pl.ds(t * TM, TM), :], wsem.at[s])

        def rcopy(t, s):
            return pltpu.make_async_copy(h_hbm.at[pl.ds(t * TM, TM), :], hbuf.at[s], rsem.at[s])

        @pl.when(p == 0)
        def _phase0():
            @pl.when(i == 0)
            def _():
                ssq_ref[...] = jnp.zeros_like(ssq_ref)

            @pl.when(i >= 2)
            def _():
                wcopy(i - 2, slot).wait()

            dw = dw_ref[...].astype(jnp.float32)
            for s in range(TM // SUB):
                xt = x_ref[pl.ds(s * SUB, SUB), :].astype(jnp.float32)
                y = xt * dw
                m = jnp.mean(y, axis=-1, keepdims=True)
                d = y - m
                v = jnp.mean(d * d, axis=-1, keepdims=True)
                xn = (d * (KS * jax.lax.rsqrt(v + 1e-5))).astype(jnp.bfloat16)
                for c in range(1536 // NCH):
                    a = jnp.dot(xn, w1_ref[:, c * NCH:(c + 1) * NCH], preferred_element_type=jnp.float32)
                    t = jnp.tanh(a * (a * a + A_LIN))
                    h = a * (t + 1.0)
                    hh = (h * h).reshape(SUB // 8, 8, NCH).sum(axis=0)
                    ssq_ref[:, c * NCH:(c + 1) * NCH] += hh
                    hbuf[slot, pl.ds(s * SUB, SUB), c * NCH:(c + 1) * NCH] = h.astype(jnp.bfloat16)
            wcopy(i, slot).start()

            @pl.when(i == n - 1)
            def _():
                wcopy(i - 1, 1 - slot).wait()
                wcopy(i, slot).wait()
                rcopy(0, 0).start()
                ss = jnp.sum(ssq_ref[...], axis=0, keepdims=True) * (H_SCALE * H_SCALE)
                gx = jnp.sqrt(ss + 1e-6)
                nx = gx / (jnp.mean(gx, axis=-1, keepdims=True) + 1e-6)
                sc = (g_ref[...].astype(jnp.float32) * nx + 1.0) * H_SCALE
                sct = jnp.transpose(jnp.broadcast_to(sc, (128, 1536)))
                for c in range(3):
                    w2s_ref[:, c * 128:(c + 1) * 128] = (
                        w2_ref[:, c * 128:(c + 1) * 128].astype(jnp.float32) * sct).astype(jnp.bfloat16)
                bb = jnp.broadcast_to(b_ref[...], (8, 1536))
                bias_ref[...] = jnp.dot(bb, w2_ref[...], preferred_element_type=jnp.float32)

        @pl.when(p == 1)
        def _phase1():
            @pl.when(i + 1 < n)
            def _():
                rcopy(i + 1, 1 - slot).start()
            rcopy(i, slot).wait()
            bias = bias_ref[0:1, :]
            for s in range(TM // SUB):
                acc = jnp.dot(hbuf[slot, pl.ds(s * SUB, SUB), :], w2s_ref[...], preferred_element_type=jnp.float32)
                o_ref[pl.ds(s * SUB, SUB), :] = (
                    acc + bias + x_ref[pl.ds(s * SUB, SUB), :].astype(jnp.float32)).astype(o_ref.dtype)

    @jax.jit
    def f(x, dw, w1, w2, grn_g, grn_b):
        B, H, W, C = x.shape
        N = B * H * W
        F = w1.shape[1]
        x2 = x.reshape(N, C)
        nt = N // TM
        out, _ = pl.pallas_call(
            kernel,
            grid=(2, nt),
            in_specs=[
                pl.BlockSpec((TM, C), lambda p, i: (i, 0)),
                pl.BlockSpec((1, C), lambda p, i: (0, 0)),
                pl.BlockSpec((C, F), lambda p, i: (0, 0)),
                pl.BlockSpec((F, C), lambda p, i: (0, 0)),
                pl.BlockSpec((1, F), lambda p, i: (0, 0)),
                pl.BlockSpec((1, F), lambda p, i: (0, 0)),
            ],
            out_specs=[
                pl.BlockSpec((TM, C), lambda p, i: (i * p, 0)),
                pl.BlockSpec(memory_space=pl.ANY),
            ],
            out_shape=[
                jax.ShapeDtypeStruct((N, C), x.dtype),
                jax.ShapeDtypeStruct((N, F), jnp.bfloat16),
            ],
            scratch_shapes=[
                pltpu.VMEM((2, TM, F), jnp.bfloat16),
                pltpu.VMEM((8, F), jnp.float32),
                pltpu.VMEM((F, C), jnp.bfloat16),
                pltpu.VMEM((8, C), jnp.float32),
                pltpu.SemaphoreType.DMA((2,)),
                pltpu.SemaphoreType.DMA((2,)),
            ],
            compiler_params=pltpu.CompilerParams(
                dimension_semantics=("arbitrary", "arbitrary"),
                vmem_limit_bytes=vmem * 1024 * 1024),
        )(x2, dw.reshape(1, C), w1, w2, grn_g.reshape(1, F), grn_b.reshape(1, F))
        return out.reshape(B, H, W, C)
    return f


_impl = make(TM=2048, SUB=256, NCH=512)


@jax.jit
def pallas_standalone__modern_conv_block_slak__vision_kernel(x, dw, w1, w2, grn_g, grn_b):
    return _impl(x, dw, w1, w2, grn_g, grn_b)
```

```python
import functools
import jax, jax.numpy as jnp
from jax.experimental import pallas as pl
from jax.experimental.pallas import tpu as pltpu

C_TANH = 0.7978845608028654
C_CUBE = 0.044715
KS = (C_TANH * C_CUBE) ** (1.0 / 3.0)
A_LIN = C_TANH / KS
H_SCALE = 0.5 / KS


def make(TM=2304, SUB=256, NCH=512, RR=512, NB=2, SUB2=None, vmem=127, pipe_ln=True, mode="both"):
    SUB2 = SUB2 or SUB
    SR = TM - RR
    NS = TM // SUB
    assert TM % SUB == 0

    def pieces(lo, hi):
        out = []
        if lo < SR:
            out.append((False, lo, min(hi, SR)))
        if hi > SR:
            out.append((True, max(lo, SR), hi))
        return out

    def kernel(x_ref, xnx_ref, dw_ref, w1_ref, w2_ref, g_ref, b_ref, o_ref, h_hbm,
               hbuf, hres, xn0_ref, ssq_ref, w2s_ref, bias_ref, wsem, rsem):
        p = pl.program_id(0) if mode == "both" else int(mode)
        i = pl.program_id(1)
        n = pl.num_programs(1)

        def wcopy(t, s):
            return pltpu.make_async_copy(hbuf.at[s], h_hbm.at[pl.ds(pl.multiple_of(t * SR, 16), SR), :], wsem.at[s])

        def rcopy(t, s):
            return pltpu.make_async_copy(h_hbm.at[pl.ds(pl.multiple_of(t * SR, 16), SR), :], hbuf.at[s], rsem.at[s])

        def ln(xt, dw):
            y = xt.astype(jnp.float32) * dw
            m = jnp.mean(y, axis=-1, keepdims=True)
            d = y - m
            v = jnp.mean(d * d, axis=-1, keepdims=True)
            return (d * (KS * jax.lax.rsqrt(v + 1e-5))).astype(jnp.bfloat16)

        def phase0():
            slot = i % NB
            dw = dw_ref[...].astype(jnp.float32)

            @pl.when(i == 0)
            def _():
                ssq_ref[...] = jnp.zeros_like(ssq_ref)
                if pipe_ln:
                    xn0_ref[...] = ln(x_ref[pl.ds(0, SUB), :], dw)

            @pl.when(i >= NB)
            def _():
                wcopy(i - NB, slot).wait()

            rbase = pl.multiple_of(i * RR, 16)
            for s in range(NS):
                if s == 0 and pipe_ln:
                    xn = xn0_ref[...]
                else:
                    xn = ln(x_ref[pl.ds(s * SUB, SUB), :], dw)
                for c in range(1536 // NCH):
                    a = jnp.dot(xn, w1_ref[:, c * NCH:(c + 1) * NCH], preferred_element_type=jnp.float32)
                    t = jnp.tanh(a * (a * a + A_LIN))
                    h = a * (t + 1.0)
                    hh = (h * h).reshape(SUB // 8, 8, NCH).sum(axis=0)
                    ssq_ref[:, c * NCH:(c + 1) * NCH] += hh
                    hb = h.astype(jnp.bfloat16)
                    for res, lo, hi in pieces(s * SUB, (s + 1) * SUB):
                        v = hb[lo - s * SUB:hi - s * SUB, :]
                        if res:
                            hres[pl.ds(rbase + (lo - SR), hi - lo), c * NCH:(c + 1) * NCH] = v
                        else:
                            hbuf[slot, pl.ds(lo, hi - lo), c * NCH:(c + 1) * NCH] = v
            if pipe_ln:
                xn0_ref[...] = ln(xnx_ref[...], dw)

            @pl.when(i < n - NB)
            def _():
                wcopy(i, slot).start()

            @pl.when(i == n - 1)
            def _():
                ss = jnp.sum(ssq_ref[...], axis=0, keepdims=True) * (H_SCALE * H_SCALE)
                gx = jnp.sqrt(ss + 1e-6)
                nx = gx / (jnp.mean(gx, axis=-1, keepdims=True) + 1e-6)
                sc = (g_ref[...].astype(jnp.float32) * nx + 1.0) * H_SCALE
                sct = jnp.transpose(jnp.broadcast_to(sc, (128, 1536)))
                for c in range(3):
                    w2s_ref[:, c * 128:(c + 1) * 128] = (
                        w2_ref[:, c * 128:(c + 1) * 128].astype(jnp.float32) * sct).astype(jnp.bfloat16)
                bb = jnp.broadcast_to(b_ref[...], (8, 1536))
                bias_ref[...] = jnp.dot(bb, w2_ref[...], preferred_element_type=jnp.float32)

        def phase1():
            t = n - 1 - i
            slot = t % NB

            @pl.when(jnp.logical_and(i >= 1, t - (NB - 1) >= 0))
            def _():
                rcopy(t - (NB - 1), (t + 1) % NB).start()

            @pl.when(i >= NB)
            def _():
                rcopy(t, slot).wait()
            bias = bias_ref[0:1, :]
            rbase = pl.multiple_of(t * RR, 16)
            lo = SR
            while lo < TM:
                hi = min(lo + SUB2, TM)
                acc = jnp.dot(hres[pl.ds(rbase + (lo - SR), hi - lo), :], w2s_ref[...], preferred_element_type=jnp.float32)
                o_ref[pl.ds(lo, hi - lo), :] = (
                    acc + bias + x_ref[pl.ds(lo, hi - lo), :].astype(jnp.float32)).astype(o_ref.dtype)
                lo = hi
            lo = 0
            while lo < SR:
                hi = min(lo + SUB2, SR)
                acc = jnp.dot(hbuf[slot, pl.ds(lo, hi - lo), :], w2s_ref[...], preferred_element_type=jnp.float32)
                o_ref[pl.ds(lo, hi - lo), :] = (
                    acc + bias + x_ref[pl.ds(lo, hi - lo), :].astype(jnp.float32)).astype(o_ref.dtype)
                lo = hi

        if mode == "both":
            pl.when(p == 0)(phase0)
            pl.when(p == 1)(phase1)
        elif mode == "0":
            phase0()
        else:
            phase1()

    @jax.jit
    def f(x, dw, w1, w2, grn_g, grn_b):
        B, H, W, C = x.shape
        N = B * H * W
        F = w1.shape[1]
        x2 = x.reshape(N, C)
        nt = N // TM
        nsub = N // SUB
        if mode == "both":
            xmap = lambda p, i: (i + p * (nt - 1 - 2 * i), 0)
            xnmap = lambda p, i: (jnp.where(p == 0, jnp.minimum((i + 1) * NS, nsub - 1), nsub - 1), 0)
            omap = lambda p, i: (nt - 1 - p * i, 0)
        elif mode == "0":
            xmap = lambda p, i: (i, 0)
            xnmap = lambda p, i: (jnp.minimum((i + 1) * NS, nsub - 1), 0)
            omap = lambda p, i: (0, 0)
        else:
            xmap = lambda p, i: (nt - 1 - i, 0)
            xnmap = lambda p, i: (0, 0)
            omap = lambda p, i: (nt - 1 - i, 0)
        one = pl.Buffered(1)
        out, _ = pl.pallas_call(
            kernel,
            grid=(2 if mode == "both" else 1, nt),
            in_specs=[
                pl.BlockSpec((TM, C), xmap),
                pl.BlockSpec((SUB, C), xnmap),
                pl.BlockSpec((1, C), lambda p, i: (0, 0)),
                pl.BlockSpec((C, F), lambda p, i: (0, 0), pipeline_mode=one),
                pl.BlockSpec((F, C), lambda p, i: (0, 0), pipeline_mode=one),
                pl.BlockSpec((1, F), lambda p, i: (0, 0)),
                pl.BlockSpec((1, F), lambda p, i: (0, 0)),
            ],
            out_specs=[
                pl.BlockSpec((TM, C), omap),
                pl.BlockSpec(memory_space=pl.ANY),
            ],
            out_shape=[
                jax.ShapeDtypeStruct((N, C), x.dtype),
                jax.ShapeDtypeStruct(((nt - NB) * SR, F), jnp.bfloat16),
            ],
            scratch_shapes=[
                pltpu.VMEM((NB, SR, F), jnp.bfloat16),
                pltpu.VMEM((max(nt * RR, 16), F), jnp.bfloat16),
                pltpu.VMEM((SUB, C), jnp.bfloat16),
                pltpu.VMEM((8, F), jnp.float32),
                pltpu.VMEM((F, C), jnp.bfloat16),
                pltpu.VMEM((8, C), jnp.float32),
                pltpu.SemaphoreType.DMA((NB,)),
                pltpu.SemaphoreType.DMA((NB,)),
            ],
            compiler_params=pltpu.CompilerParams(
                dimension_semantics=("arbitrary", "arbitrary"),
                vmem_limit_bytes=vmem * 1024 * 1024),
        )(x2, x2, dw.reshape(1, C), w1, w2, grn_g.reshape(1, F), grn_b.reshape(1, F))
        return out.reshape(B, H, W, C)
    return f


_impl = make()


@jax.jit
def pallas_standalone__modern_conv_block_slak__vision_kernel(x, dw, w1, w2, grn_g, grn_b):
    return _impl(x, dw, w1, w2, grn_g, grn_b)
```

```python
import functools
import jax, jax.numpy as jnp
from jax import lax
from jax.experimental import pallas as pl
from jax.experimental.pallas import tpu as pltpu

C_TANH = 0.7978845608028654
C_CUBE = 0.044715
KS = (C_TANH * C_CUBE) ** (1.0 / 3.0)
A_LIN = C_TANH / KS
H_SCALE = 0.5 / KS


def ranges(sizes):
    out, lo = [], 0
    for s in sizes:
        out.append((lo, lo + s)); lo += s
    return out


def make(TM=4608, SUB0=128, SUB1=256, NCH=512, RR=896, OCH=4, HCH=1, vmem=128, mode="both", nobc=True, nod=""):
    SR = TM - RR
    S0 = [SUB0] * (TM // SUB0)
    S1 = [SUB1] * (TM // SUB1)
    assert sum(S0) == TM and sum(S1) == TM
    F0 = S0[0]
    assert TM % OCH == 0 and (TM // OCH) % 16 == 0
    OR = TM // OCH
    assert SR % HCH == 0 and (SR // HCH) % 16 == 0
    HR = SR // HCH

    def pieces(lo, hi):
        out = []
        if lo < SR:
            out.append((False, lo, min(hi, SR)))
        if hi > SR:
            out.append((True, max(lo, SR), hi))
        return out

    def kernel(x_hbm, dw_ref, w1_hbm, w2_hbm, g_ref, b_ref, o_hbm, h_hbm,
               xbuf, obuf, xhead, hbuf, hres, xn0_ref, ssq_ref, w1v, w2v, bias_ref,
               xsem, xhsem, osem, hwsem, hrsem, wsem):
        n = x_hbm.shape[0] // TM

        def row0(t, rows):
            return pl.multiple_of(t * rows, 16)

        def xcopy(t, s):
            return pltpu.make_async_copy(x_hbm.at[pl.ds(row0(t, TM), TM), :], xbuf.at[s], xsem.at[s])

        def xhcopy(t, s):
            return pltpu.make_async_copy(x_hbm.at[pl.ds(row0(t, TM), F0), :], xhead.at[s], xhsem.at[s])

        def hwcopy(t, s, k):
            return pltpu.make_async_copy(hbuf.at[s, pl.ds(k * HR, HR), :],
                                         h_hbm.at[pl.ds(pl.multiple_of(t * SR + k * HR, 16), HR), :], hwsem.at[s])

        def hrcopy(t, s):
            return pltpu.make_async_copy(h_hbm.at[pl.ds(row0(t, SR), SR), :], hbuf.at[s], hrsem.at[s])

        def ocopy(t, s, k):
            return pltpu.make_async_copy(obuf.at[s, pl.ds(k * OR, OR), :],
                                         o_hbm.at[pl.ds(pl.multiple_of(t * TM + k * OR, 16), OR), :], osem.at[s])

        w1copy = pltpu.make_async_copy(w1_hbm, w1v, wsem.at[0])
        w2copy = pltpu.make_async_copy(w2_hbm, w2v, wsem.at[1])

        def ln(xt, dw):
            y = xt.astype(jnp.float32) * dw
            m = jnp.mean(y, axis=-1, keepdims=True)
            d = y - m
            v = jnp.mean(d * d, axis=-1, keepdims=True)
            return (d * (KS * lax.rsqrt(v + 1e-5))).astype(jnp.bfloat16)

        dw = dw_ref[...].astype(jnp.float32)

        xhcopy(0, 0).start()
        w1copy.start()
        xcopy(0, 0).start()
        xhcopy(1, 1).start()
        w2copy.start()
        ssq_ref[...] = jnp.zeros_like(ssq_ref)
        xhcopy(0, 0).wait()
        xn0_ref[...] = ln(xhead[0], dw)
        w1copy.wait()

        def body0(i, carry):
            slot = i % 2
            xcopy(i, slot).wait()

            @pl.when(i + 1 < n)
            def _():
                xcopy(i + 1, 1 - slot).start()
                xhcopy(i + 1, 1 - slot).wait()

            @pl.when(i + 2 < n)
            def _():
                xhcopy(i + 2, slot).start()

            @pl.when(i >= 2)
            def _():
                for k in range(HCH):
                    hwcopy(i - 2, slot, k).wait()

            rbase = pl.multiple_of(i * RR, 16)
            hnext = 0
            for s, (r0, r1) in enumerate(ranges(S0)):
                R = r1 - r0
                if s == 0:
                    xn = xn0_ref[...]
                else:
                    xn = ln(xbuf[slot, pl.ds(r0, R), :], dw)
                for c in range(1536 // NCH):
                    a = jnp.dot(xn, w1v[:, c * NCH:(c + 1) * NCH], preferred_element_type=jnp.float32)
                    t = jnp.tanh(a * (a * a + A_LIN))
                    h = a * (t + 1.0)
                    hh = (h * h).reshape(R // 8, 8, NCH).sum(axis=0)
                    ssq_ref[:, c * NCH:(c + 1) * NCH] += hh
                    hb = h.astype(jnp.bfloat16)
                    for res, lo, hi in pieces(r0, r1):
                        v = hb[lo - r0:hi - r0, :]
                        if res:
                            hres[pl.ds(rbase + (lo - SR), hi - lo), c * NCH:(c + 1) * NCH] = v
                        else:
                            hbuf[slot, pl.ds(lo, hi - lo), c * NCH:(c + 1) * NCH] = v
                while hnext < HCH and (hnext + 1) * HR <= r1:
                    kk = hnext

                    @pl.when(i < n - 2)
                    def _():
                        hwcopy(i, slot, kk).start()
                    hnext += 1
            xn0_ref[...] = ln(xhead[1 - slot], dw)
            return carry

        if mode in ("both", "0"):
            lax.fori_loop(0, n, body0, 0)
        else:
            xcopy(0, 0).wait()
            xhcopy(1, 1).wait()

        w2copy.wait()
        ss = jnp.sum(ssq_ref[...], axis=0, keepdims=True) * (H_SCALE * H_SCALE)
        gx = jnp.sqrt(ss + 1e-6)
        nx = gx / (jnp.mean(gx, axis=-1, keepdims=True) + 1e-6)
        sc = (g_ref[...].astype(jnp.float32) * nx + 1.0) * H_SCALE
        sct = jnp.transpose(jnp.broadcast_to(sc, (128, 1536)))
        bb = jnp.broadcast_to(b_ref[...], (8, 1536))
        bias_ref[...] = jnp.dot(bb, w2v[...], preferred_element_type=jnp.float32)
        for c in range(3):
            w2v[:, c * 128:(c + 1) * 128] = (
                w2v[:, c * 128:(c + 1) * 128].astype(jnp.float32) * sct).astype(jnp.bfloat16)

        def body1(j, carry):
            t = n - 1 - j
            slot = t % 2

            @pl.when(j >= 2)
            def _():
                if "x" not in nod: xcopy(t, slot).wait()
                if "h" not in nod: hrcopy(t, slot).wait()
                for k in range(OCH):
                    if "o" not in nod: ocopy(t + 2, slot, k).wait()

            @pl.when(jnp.logical_and(j >= 1, t >= 1))
            def _():
                if "h" not in nod: hrcopy(t - 1, 1 - slot).start()
                if "x" not in nod: xcopy(t - 1, 1 - slot).start()

            bias = bias_ref[0:1, :]
            rbase = pl.multiple_of(t * RR, 16)
            onext = 0
            for (r0, r1) in ranges(S1):
                for res, lo, hi in pieces(r0, r1):
                    if res:
                        lhs = hres[pl.ds(rbase + (lo - SR), hi - lo), :]
                    else:
                        lhs = hbuf[slot, pl.ds(lo, hi - lo), :]
                    acc = jnp.dot(lhs, w2v[...], preferred_element_type=jnp.float32)
                    obuf[slot, pl.ds(lo, hi - lo), :] = (
                        acc + bias + xbuf[slot, pl.ds(lo, hi - lo), :].astype(jnp.float32)).astype(obuf.dtype)
                while onext < OCH and (onext + 1) * OR <= r1:
                    if "o" not in nod: ocopy(t, slot, onext).start()
                    onext += 1
            return carry

        if mode in ("both", "1"):
            lax.fori_loop(0, n, body1, 0)
            for t in (1, 0):
                for k in range(OCH):
                    if "o" not in nod: ocopy(t, t % 2, k).wait()
        if mode == "0":
            pass

    @jax.jit
    def f(x, dw, w1, w2, grn_g, grn_b):
        B, H, W, C = x.shape
        N = B * H * W
        F = w1.shape[1]
        x2 = x.reshape(N, C)
        nt = N // TM
        hbm = pl.BlockSpec(memory_space=pl.ANY)
        vm = pl.BlockSpec(memory_space=pltpu.VMEM)
        out, _ = pl.pallas_call(
            kernel,
            in_specs=[hbm, vm, hbm, hbm, vm, vm],
            out_specs=[hbm, hbm],
            out_shape=[
                jax.ShapeDtypeStruct((N, C), x.dtype),
                jax.ShapeDtypeStruct(((nt - 2) * SR, F), jnp.bfloat16),
            ],
            scratch_shapes=[
                pltpu.VMEM((2, TM, C), jnp.bfloat16),
                pltpu.VMEM((2, TM, C), jnp.bfloat16),
                pltpu.VMEM((2, F0, C), jnp.bfloat16),
                pltpu.VMEM((2, SR, F), jnp.bfloat16),
                pltpu.VMEM((nt * RR, F), jnp.bfloat16),
                pltpu.VMEM((F0, C), jnp.bfloat16),
                pltpu.VMEM((8, F), jnp.float32),
                pltpu.VMEM((C, F), jnp.bfloat16),
                pltpu.VMEM((F, C), jnp.bfloat16),
                pltpu.VMEM((8, C), jnp.float32),
                pltpu.SemaphoreType.DMA((2,)),
                pltpu.SemaphoreType.DMA((2,)),
                pltpu.SemaphoreType.DMA((2,)),
                pltpu.SemaphoreType.DMA((2,)),
                pltpu.SemaphoreType.DMA((2,)),
                pltpu.SemaphoreType.DMA((2,)),
            ],
            compiler_params=pltpu.CompilerParams(
                vmem_limit_bytes=vmem * 1024 * 1024, disable_bounds_checks=nobc),
        )(x2, dw.reshape(1, C), w1, w2, grn_g.reshape(1, F), grn_b.reshape(1, F))
        return out.reshape(B, H, W, C)
    return f


_impl = make(TM=3072, RR=672)


@jax.jit
def pallas_standalone__modern_conv_block_slak__vision_kernel(x, dw, w1, w2, grn_g, grn_b):
    return _impl(x, dw, w1, w2, grn_g, grn_b)
```

```python
import functools
import jax, jax.numpy as jnp
from jax import lax
from jax.experimental import pallas as pl
from jax.experimental.pallas import tpu as pltpu

C_TANH = 0.7978845608028654
C_CUBE = 0.044715
KS = (C_TANH * C_CUBE) ** (1.0 / 3.0)
A_LIN = C_TANH / KS
H_SCALE = 0.5 / KS


def ranges(total, size):
    out, lo = [], 0
    while lo < total:
        hi = min(lo + size, total)
        out.append((lo, hi)); lo = hi
    return out


def make(TM=3584, REM=512, MS=256, SUB0=128, SUB1=256, NCH=512, RR=768, OCHS=None, vmem=128,
         nobc=True, nosc=True):
    SR = TM - RR
    F0 = SUB0
    NM = REM // MS if REM else 0
    if OCHS is None:
        q = (TM // 4) // SUB1 * SUB1
        OCHS = [q, q, q, TM - 3 * q]
    assert sum(OCHS) == TM
    ORG = []
    lo = 0
    for c in OCHS:
        ORG.append((lo, lo + c)); lo += c

    def pieces(lo, hi):
        out = []
        if lo < SR:
            out.append((False, lo, min(hi, SR)))
        if hi > SR:
            out.append((True, max(lo, SR), hi))
        return out

    def kernel(x_hbm, dw_hbm, w1_hbm, w2_hbm, g_hbm, b_hbm, o_hbm, h_hbm,
               xbuf, obuf, xhead, hbuf, hres, xrem, hrem, orem, xn0_ref, ssq_ref, w1v, w2v, bias_ref,
               dw_ref, g_ref, b_ref,
               xsem, xhsem, osem, hwsem, hrsem, wsem, rsem):
        n = (x_hbm.shape[0] - REM) // TM

        def al(v):
            return pl.multiple_of(v, 16)

        def xcopy(t, s):
            return pltpu.make_async_copy(x_hbm.at[pl.ds(al(REM + t * TM), TM), :], xbuf.at[s], xsem.at[s])

        def xhcopy(t, s):
            return pltpu.make_async_copy(x_hbm.at[pl.ds(al(REM + t * TM), F0), :], xhead.at[s], xhsem.at[s])

        def hwcopy(t, s):
            return pltpu.make_async_copy(hbuf.at[s], h_hbm.at[pl.ds(al(t * SR), SR), :], hwsem.at[s])

        def hrcopy(t, s):
            return pltpu.make_async_copy(h_hbm.at[pl.ds(al(t * SR), SR), :], hbuf.at[s], hrsem.at[s])

        def ocopy(t, s, k):
            lo, hi = ORG[k]
            return pltpu.make_async_copy(obuf.at[s, pl.ds(lo, hi - lo), :],
                                         o_hbm.at[pl.ds(al(REM + t * TM + lo), hi - lo), :], osem.at[s])

        def orcopy(k):
            return pltpu.make_async_copy(orem.at[pl.ds(al(k * MS), MS), :],
                                         o_hbm.at[pl.ds(al(k * MS), MS), :], rsem.at[1])

        w1copy = pltpu.make_async_copy(w1_hbm, w1v, wsem.at[0])
        w2copy = pltpu.make_async_copy(w2_hbm, w2v, wsem.at[1])
        dwcopy = pltpu.make_async_copy(dw_hbm, dw_ref, wsem.at[2])
        gcopy = pltpu.make_async_copy(g_hbm, g_ref, wsem.at[3])
        bcopy = pltpu.make_async_copy(b_hbm, b_ref, wsem.at[4])
        xrcopy = pltpu.make_async_copy(x_hbm.at[pl.ds(0, REM + F0), :], xrem, rsem.at[0])

        def ln(xt, dw):
            y = xt.astype(jnp.float32) * dw
            m = jnp.mean(y, axis=-1, keepdims=True)
            d = y - m
            v = jnp.mean(d * d, axis=-1, keepdims=True)
            return (d * (KS * lax.rsqrt(v + 1e-5))).astype(jnp.bfloat16)

        def expand(xn, put):
            R = xn.shape[0]
            for c in range(1536 // NCH):
                a = jnp.dot(xn, w1v[:, c * NCH:(c + 1) * NCH], preferred_element_type=jnp.float32)
                t = jnp.tanh(a * (a * a + A_LIN))
                h = a * (t + 1.0)
                hh = (h * h).reshape(R // 8, 8, NCH).sum(axis=0)
                ssq_ref[:, c * NCH:(c + 1) * NCH] += hh
                put(c, h.astype(jnp.bfloat16))

        dwcopy.start()
        xrcopy.start()
        w1copy.start()
        xcopy(0, 0).start()
        xhcopy(1, 1).start()
        ssq_ref[...] = jnp.zeros_like(ssq_ref)
        dwcopy.wait()
        dw = dw_ref[...].astype(jnp.float32)
        xrcopy.wait()
        xn0_ref[...] = ln(xrem[pl.ds(0, F0), :], dw)
        w1copy.wait()

        def mini0(k, carry):
            base = pl.multiple_of(k * MS, MS)
            for (r0, r1) in ranges(MS, SUB0):
                R = r1 - r0
                if r0 == 0:
                    xn = xn0_ref[...]
                else:
                    xn = ln(xrem[pl.ds(base + r0, R), :], dw)

                def put(c, hb):
                    hrem[pl.ds(base + r0, R), c * NCH:(c + 1) * NCH] = hb
                expand(xn, put)
            xn0_ref[...] = ln(xrem[pl.ds(base + MS, F0), :], dw)
            return carry

        if NM:
            lax.fori_loop(0, NM, mini0, 0)

        def body0(i, carry):
            slot = i & 1
            nslot = 1 - slot

            @pl.when(i >= 2)
            def _():
                hwcopy(i - 2, slot).wait()

            xcopy(i, slot).wait()

            @pl.when(i + 1 < n)
            def _():
                xhcopy(i + 1, nslot).wait()

            @pl.when(i + 1 < n)
            def _():
                xcopy(i + 1, nslot).start()

            @pl.when(i + 2 < n)
            def _():
                xhcopy(i + 2, slot).start()

            @pl.when(i == 1)
            def _():
                w2copy.start()
                gcopy.start()
                bcopy.start()

            rbase = al(i * RR)
            for (r0, r1) in ranges(TM, SUB0):
                R = r1 - r0
                if r0 == 0:
                    xn = xn0_ref[...]
                else:
                    xn = ln(xbuf[slot, pl.ds(r0, R), :], dw)

                def put(c, hb):
                    for res, lo, hi in pieces(r0, r1):
                        v = hb[lo - r0:hi - r0, :]
                        if res:
                            hres[pl.ds(rbase + (lo - SR), hi - lo), c * NCH:(c + 1) * NCH] = v
                        else:
                            hbuf[slot, pl.ds(lo, hi - lo), c * NCH:(c + 1) * NCH] = v
                expand(xn, put)
                if r0 < SR <= r1:
                    @pl.when(i < n - 2)
                    def _():
                        hwcopy(i, slot).start()
            xn0_ref[...] = ln(xhead[nslot], dw)
            return carry

        lax.fori_loop(0, n, body0, 0)

        w2copy.wait()
        gcopy.wait()
        bcopy.wait()
        ss = jnp.sum(ssq_ref[...], axis=0, keepdims=True) * (H_SCALE * H_SCALE)
        gx = jnp.sqrt(ss + 1e-6)
        nx = gx / (jnp.mean(gx, axis=-1, keepdims=True) + 1e-6)
        g = g_ref[...].reshape(1, 1536)
        b = b_ref[...].reshape(1, 1536)
        sc = (g.astype(jnp.float32) * nx + 1.0) * H_SCALE
        bb = jnp.broadcast_to(b, (8, 1536))
        bias_ref[...] = jnp.dot(bb, w2v[...], preferred_element_type=jnp.float32)
        for r in range(12):
            sct = jnp.transpose(jnp.broadcast_to(sc[:, r * 128:(r + 1) * 128], (128, 128)))
            for c in range(3):
                w2v[r * 128:(r + 1) * 128, c * 128:(c + 1) * 128] = (
                    w2v[r * 128:(r + 1) * 128, c * 128:(c + 1) * 128].astype(jnp.float32) * sct).astype(jnp.bfloat16)

        def contract(lhs, xres):
            acc = jnp.dot(lhs, w2v[...], preferred_element_type=jnp.float32)
            return (acc + bias_ref[0:1, :] + xres.astype(jnp.float32)).astype(jnp.bfloat16)

        def body1(j, carry):
            t = n - 1 - j
            slot = t & 1
            nslot = 1 - slot

            @pl.when(j >= 2)
            def _():
                hrcopy(t, slot).wait()
                xcopy(t, slot).wait()
                for k in range(len(ORG)):
                    ocopy(t + 2, slot, k).wait()

            @pl.when(jnp.logical_and(j >= 1, t >= 1))
            def _():
                hrcopy(t - 1, nslot).start()
                xcopy(t - 1, nslot).start()

            rbase = al(t * RR)
            onext = 0
            for (r0, r1) in ranges(TM, SUB1):
                for res, lo, hi in pieces(r0, r1):
                    if res:
                        lhs = hres[pl.ds(rbase + (lo - SR), hi - lo), :]
                    else:
                        lhs = hbuf[slot, pl.ds(lo, hi - lo), :]
                    obuf[slot, pl.ds(lo, hi - lo), :] = contract(lhs, xbuf[slot, pl.ds(lo, hi - lo), :])
                while onext < len(ORG) and ORG[onext][1] <= r1:
                    ocopy(t, slot, onext).start()
                    onext += 1
            return carry

        lax.fori_loop(0, n, body1, 0)

        def mini1(k, carry):
            base = pl.multiple_of(k * MS, MS)
            for (r0, r1) in ranges(MS, SUB1):
                R = r1 - r0
                orem[pl.ds(base + r0, R), :] = contract(hrem[pl.ds(base + r0, R), :], xrem[pl.ds(base + r0, R), :])
            orcopy(k).start()
            return carry

        if NM:
            lax.fori_loop(0, NM, mini1, 0)
        for t in (1, 0):
            for k in range(len(ORG)):
                ocopy(t, t % 2, k).wait()
        for k in range(NM):
            orcopy(k).wait()

    @jax.jit
    def f(x, dw, w1, w2, grn_g, grn_b):
        B, H, W, C = x.shape
        N = B * H * W
        F = w1.shape[1]
        x2 = x.reshape(N, C)
        nt = (N - REM) // TM
        assert REM + nt * TM == N
        hbm = pl.BlockSpec(memory_space=pl.ANY)
        out, _ = pl.pallas_call(
            kernel,
            in_specs=[hbm] * 6,
            out_specs=[hbm, hbm],
            out_shape=[
                jax.ShapeDtypeStruct((N, C), x.dtype),
                jax.ShapeDtypeStruct(((nt - 2) * SR, F), jnp.bfloat16),
            ],
            scratch_shapes=[
                pltpu.VMEM((2, TM, C), jnp.bfloat16),
                pltpu.VMEM((2, TM, C), jnp.bfloat16),
                pltpu.VMEM((2, F0, C), jnp.bfloat16),
                pltpu.VMEM((2, SR, F), jnp.bfloat16),
                pltpu.VMEM((nt * RR, F), jnp.bfloat16),
                pltpu.VMEM((REM + F0, C), jnp.bfloat16),
                pltpu.VMEM((max(REM, 16), F), jnp.bfloat16),
                pltpu.VMEM((max(REM, 16), C), jnp.bfloat16),
                pltpu.VMEM((F0, C), jnp.bfloat16),
                pltpu.VMEM((8, F), jnp.float32),
                pltpu.VMEM((C, F), jnp.bfloat16),
                pltpu.VMEM((F, C), jnp.bfloat16),
                pltpu.VMEM((8, C), jnp.float32),
                pltpu.VMEM((1, C), jnp.bfloat16),
                pltpu.VMEM((F,), jnp.bfloat16),
                pltpu.VMEM((F,), jnp.bfloat16),
                pltpu.SemaphoreType.DMA((2,)),
                pltpu.SemaphoreType.DMA((2,)),
                pltpu.SemaphoreType.DMA((2,)),
                pltpu.SemaphoreType.DMA((2,)),
                pltpu.SemaphoreType.DMA((2,)),
                pltpu.SemaphoreType.DMA((5,)),
                pltpu.SemaphoreType.DMA((2,)),
            ],
            compiler_params=pltpu.CompilerParams(
                vmem_limit_bytes=vmem * 1024 * 1024, disable_bounds_checks=nobc,
                disable_semaphore_checks=nosc),
        )(x2, dw.reshape(1, C), w1, w2, grn_g, grn_b)
        return out.reshape(B, H, W, C)
    return f


_impl = make()


@jax.jit
def pallas_standalone__modern_conv_block_slak__vision_kernel(x, dw, w1, w2, grn_g, grn_b):
    return _impl(x, dw, w1, w2, grn_g, grn_b)
```

```python
import functools
import jax, jax.numpy as jnp
from jax import lax
from jax.experimental import pallas as pl
from jax.experimental.pallas import tpu as pltpu

C_TANH = 0.7978845608028654
C_CUBE = 0.044715
KS = (C_TANH * C_CUBE) ** (1.0 / 3.0)
A_LIN = C_TANH / KS
H_SCALE = 0.5 / KS


def ranges(total, size):
    out, lo = [], 0
    while lo < total:
        hi = min(lo + size, total)
        out.append((lo, hi)); lo = hi
    return out


def make(TM=3584, REM=512, MS=256, SUB0=64, SUB1=256, NCH=256, RR=768, OCHS=None, vmem=128,
         nobc=True, nosc=False, late_x0=0):
    SR = TM - RR
    F0 = SUB0
    NM = REM // MS if REM else 0
    if OCHS is None:
        q = (TM // 4) // SUB1 * SUB1
        OCHS = [q, q, q, TM - 3 * q]
    assert sum(OCHS) == TM
    ORG = []
    lo = 0
    for c in OCHS:
        ORG.append((lo, lo + c)); lo += c

    def pieces(lo, hi):
        out = []
        if lo < SR:
            out.append((False, lo, min(hi, SR)))
        if hi > SR:
            out.append((True, max(lo, SR), hi))
        return out

    def kernel(x_hbm, dw_hbm, w1_hbm, w2_hbm, g_hbm, b_hbm, o_hbm, h_hbm,
               xbuf, obuf, xhead, hbuf, hres, xrem, hrem, orem, xn0_ref, ssq_ref, w1v, w2v, bias_ref,
               dw_ref, g_ref, b_ref,
               xsem, xhsem, osem, hwsem, hrsem, wsem, rsem):
        n = (x_hbm.shape[0] - REM) // TM

        def al(v):
            return pl.multiple_of(v, 16)

        def xcopy(t, s):
            return pltpu.make_async_copy(x_hbm.at[pl.ds(al(REM + t * TM), TM), :], xbuf.at[s], xsem.at[s])

        def xhcopy(t, s):
            return pltpu.make_async_copy(x_hbm.at[pl.ds(al(REM + t * TM), F0), :], xhead.at[s], xhsem.at[s])

        def hwcopy(t, s):
            return pltpu.make_async_copy(hbuf.at[s], h_hbm.at[pl.ds(al(t * SR), SR), :], hwsem.at[s])

        def hrcopy(t, s):
            return pltpu.make_async_copy(h_hbm.at[pl.ds(al(t * SR), SR), :], hbuf.at[s], hrsem.at[s])

        def ocopy(t, s, k):
            lo, hi = ORG[k]
            return pltpu.make_async_copy(obuf.at[s, pl.ds(lo, hi - lo), :],
                                         o_hbm.at[pl.ds(al(REM + t * TM + lo), hi - lo), :], osem.at[s])

        def orcopy(k):
            return pltpu.make_async_copy(orem.at[pl.ds(al(k * MS), MS), :],
                                         o_hbm.at[pl.ds(al(k * MS), MS), :], rsem.at[1])

        w1copy = pltpu.make_async_copy(w1_hbm, w1v, wsem.at[0])
        w2copy = pltpu.make_async_copy(w2_hbm, w2v, wsem.at[1])
        dwcopy = pltpu.make_async_copy(dw_hbm, dw_ref, wsem.at[2])
        gcopy = pltpu.make_async_copy(g_hbm, g_ref, wsem.at[3])
        bcopy = pltpu.make_async_copy(b_hbm, b_ref, wsem.at[4])
        xrcopy = pltpu.make_async_copy(x_hbm.at[pl.ds(0, REM + F0), :], xrem, rsem.at[0])

        def ln(xt, dw):
            y = xt.astype(jnp.float32) * dw
            m = jnp.mean(y, axis=-1, keepdims=True)
            d = y - m
            v = jnp.mean(d * d, axis=-1, keepdims=True)
            return (d * (KS * lax.rsqrt(v + 1e-5))).astype(jnp.bfloat16)

        def expand(xn, put):
            R = xn.shape[0]
            for c in range(1536 // NCH):
                a = jnp.dot(xn, w1v[:, c * NCH:(c + 1) * NCH], preferred_element_type=jnp.float32)
                t = jnp.tanh(a * (a * a + A_LIN))
                h = a * (t + 1.0)
                hh = (h * h).reshape(R // 8, 8, NCH).sum(axis=0)
                ssq_ref[:, c * NCH:(c + 1) * NCH] += hh
                put(c, h.astype(jnp.bfloat16))

        dwcopy.start()
        xrcopy.start()
        w1copy.start()
        if late_x0 == 0:
            xcopy(0, 0).start()
            xhcopy(1, 1).start()
        ssq_ref[...] = jnp.zeros_like(ssq_ref)
        dwcopy.wait()
        dw = dw_ref[...].astype(jnp.float32)
        xrcopy.wait()
        if late_x0 == 2:
            xcopy(0, 0).start()
            xhcopy(1, 1).start()
        xn0_ref[...] = ln(xrem[pl.ds(0, F0), :], dw)
        w1copy.wait()
        if late_x0 == 1:
            xcopy(0, 0).start()
            xhcopy(1, 1).start()

        def mini0(k, carry):
            base = pl.multiple_of(k * MS, MS)
            for (r0, r1) in ranges(MS, SUB0):
                R = r1 - r0
                if r0 == 0:
                    xn = xn0_ref[...]
                else:
                    xn = ln(xrem[pl.ds(base + r0, R), :], dw)

                def put(c, hb):
                    hrem[pl.ds(base + r0, R), c * NCH:(c + 1) * NCH] = hb
                expand(xn, put)
            xn0_ref[...] = ln(xrem[pl.ds(base + MS, F0), :], dw)
            return carry

        if NM:
            lax.fori_loop(0, NM, mini0, 0)

        def body0(i, carry):
            slot = i & 1
            nslot = 1 - slot

            @pl.when(i >= 2)
            def _():
                hwcopy(i - 2, slot).wait()

            xcopy(i, slot).wait()

            @pl.when(i + 1 < n)
            def _():
                xhcopy(i + 1, nslot).wait()

            @pl.when(i + 1 < n)
            def _():
                xcopy(i + 1, nslot).start()

            @pl.when(i + 2 < n)
            def _():
                xhcopy(i + 2, slot).start()

            @pl.when(i == 1)
            def _():
                w2copy.start()
                gcopy.start()
                bcopy.start()

            rbase = al(i * RR)
            for (r0, r1) in ranges(TM, SUB0):
                R = r1 - r0
                if r0 == 0:
                    xn = xn0_ref[...]
                else:
                    xn = ln(xbuf[slot, pl.ds(r0, R), :], dw)

                def put(c, hb):
                    for res, lo, hi in pieces(r0, r1):
                        v = hb[lo - r0:hi - r0, :]
                        if res:
                            hres[pl.ds(rbase + (lo - SR), hi - lo), c * NCH:(c + 1) * NCH] = v
                        else:
                            hbuf[slot, pl.ds(lo, hi - lo), c * NCH:(c + 1) * NCH] = v
                expand(xn, put)
                if r0 < SR <= r1:
                    @pl.when(i < n - 2)
                    def _():
                        hwcopy(i, slot).start()
            xn0_ref[...] = ln(xhead[nslot], dw)
            return carry

        lax.fori_loop(0, n, body0, 0)

        w2copy.wait()
        gcopy.wait()
        bcopy.wait()
        ss = jnp.sum(ssq_ref[...], axis=0, keepdims=True) * (H_SCALE * H_SCALE)
        gx = jnp.sqrt(ss + 1e-6)
        nx = gx / (jnp.mean(gx, axis=-1, keepdims=True) + 1e-6)
        g = g_ref[...].reshape(1, 1536)
        b = b_ref[...].reshape(1, 1536)
        sc = (g.astype(jnp.float32) * nx + 1.0) * H_SCALE
        bb = jnp.broadcast_to(b, (8, 1536))
        bias_ref[...] = jnp.dot(bb, w2v[...], preferred_element_type=jnp.float32)
        for r in range(12):
            sct = jnp.transpose(jnp.broadcast_to(sc[:, r * 128:(r + 1) * 128], (128, 128)))
            for c in range(3):
                w2v[r * 128:(r + 1) * 128, c * 128:(c + 1) * 128] = (
                    w2v[r * 128:(r + 1) * 128, c * 128:(c + 1) * 128].astype(jnp.float32) * sct).astype(jnp.bfloat16)

        def contract(lhs, xres):
            acc = jnp.dot(lhs, w2v[...], preferred_element_type=jnp.float32)
            return (acc + bias_ref[0:1, :] + xres.astype(jnp.float32)).astype(jnp.bfloat16)

        def body1(j, carry):
            t = n - 1 - j
            slot = t & 1
            nslot = 1 - slot

            @pl.when(j >= 2)
            def _():
                hrcopy(t, slot).wait()
                xcopy(t, slot).wait()
                for k in range(len(ORG)):
                    ocopy(t + 2, slot, k).wait()

            @pl.when(jnp.logical_and(j >= 1, t >= 1))
            def _():
                hrcopy(t - 1, nslot).start()
                xcopy(t - 1, nslot).start()

            rbase = al(t * RR)
            onext = 0
            for (r0, r1) in ranges(TM, SUB1):
                for res, lo, hi in pieces(r0, r1):
                    if res:
                        lhs = hres[pl.ds(rbase + (lo - SR), hi - lo), :]
                    else:
                        lhs = hbuf[slot, pl.ds(lo, hi - lo), :]
                    obuf[slot, pl.ds(lo, hi - lo), :] = contract(lhs, xbuf[slot, pl.ds(lo, hi - lo), :])
                while onext < len(ORG) and ORG[onext][1] <= r1:
                    ocopy(t, slot, onext).start()
                    onext += 1
            return carry

        lax.fori_loop(0, n, body1, 0)

        def mini1(k, carry):
            base = pl.multiple_of(k * MS, MS)
            for (r0, r1) in ranges(MS, SUB1):
                R = r1 - r0
                orem[pl.ds(base + r0, R), :] = contract(hrem[pl.ds(base + r0, R), :], xrem[pl.ds(base + r0, R), :])
            orcopy(k).start()
            return carry

        if NM:
            lax.fori_loop(0, NM, mini1, 0)
        for t in (1, 0):
            for k in range(len(ORG)):
                ocopy(t, t % 2, k).wait()
        for k in range(NM):
            orcopy(k).wait()

    @jax.jit
    def f(x, dw, w1, w2, grn_g, grn_b):
        B, H, W, C = x.shape
        N = B * H * W
        F = w1.shape[1]
        x2 = x.reshape(N, C)
        nt = (N - REM) // TM
        assert REM + nt * TM == N
        hbm = pl.BlockSpec(memory_space=pl.ANY)
        out, _ = pl.pallas_call(
            kernel,
            in_specs=[hbm] * 6,
            out_specs=[hbm, hbm],
            out_shape=[
                jax.ShapeDtypeStruct((N, C), x.dtype),
                jax.ShapeDtypeStruct(((nt - 2) * SR, F), jnp.bfloat16),
            ],
            scratch_shapes=[
                pltpu.VMEM((2, TM, C), jnp.bfloat16),
                pltpu.VMEM((2, TM, C), jnp.bfloat16),
                pltpu.VMEM((2, F0, C), jnp.bfloat16),
                pltpu.VMEM((2, SR, F), jnp.bfloat16),
                pltpu.VMEM((nt * RR, F), jnp.bfloat16),
                pltpu.VMEM((REM + F0, C), jnp.bfloat16),
                pltpu.VMEM((max(REM, 16), F), jnp.bfloat16),
                pltpu.VMEM((max(REM, 16), C), jnp.bfloat16),
                pltpu.VMEM((F0, C), jnp.bfloat16),
                pltpu.VMEM((8, F), jnp.float32),
                pltpu.VMEM((C, F), jnp.bfloat16),
                pltpu.VMEM((F, C), jnp.bfloat16),
                pltpu.VMEM((8, C), jnp.float32),
                pltpu.VMEM((1, C), jnp.bfloat16),
                pltpu.VMEM((F,), jnp.bfloat16),
                pltpu.VMEM((F,), jnp.bfloat16),
                pltpu.SemaphoreType.DMA((2,)),
                pltpu.SemaphoreType.DMA((2,)),
                pltpu.SemaphoreType.DMA((2,)),
                pltpu.SemaphoreType.DMA((2,)),
                pltpu.SemaphoreType.DMA((2,)),
                pltpu.SemaphoreType.DMA((5,)),
                pltpu.SemaphoreType.DMA((2,)),
            ],
            compiler_params=pltpu.CompilerParams(
                vmem_limit_bytes=vmem * 1024 * 1024, disable_bounds_checks=nobc,
                disable_semaphore_checks=nosc),
        )(x2, dw.reshape(1, C), w1, w2, grn_g, grn_b)
        return out.reshape(B, H, W, C)
    return f


_impl = make()


@jax.jit
def pallas_standalone__modern_conv_block_slak__vision_kernel(x, dw, w1, w2, grn_g, grn_b):
    return _impl(x, dw, w1, w2, grn_g, grn_b)
```

```python
import jax
import jax.numpy as jnp
from jax import lax
from jax.experimental import pallas as pl
from jax.experimental.pallas import tpu as pltpu

C_TANH = 0.7978845608028654
C_CUBE = 0.044715
KS = (C_TANH * C_CUBE) ** (1.0 / 3.0)
A_LIN = C_TANH / KS
H_SCALE = 0.5 / KS

TM = 3584
REM = 512
MS = 256
SUB0 = 64
SUB1 = 256
NCH = 256
RR = 768
SR = TM - RR
NOC = 4


def _ranges(total, size):
    out, lo = [], 0
    while lo < total:
        hi = min(lo + size, total)
        out.append((lo, hi))
        lo = hi
    return out


def _pieces(lo, hi):
    out = []
    if lo < SR:
        out.append((False, lo, min(hi, SR)))
    if hi > SR:
        out.append((True, max(lo, SR), hi))
    return out


_OC = _ranges(TM, -(-TM // NOC // SUB1) * SUB1)


def _kernel(x_hbm, dw_hbm, w1_hbm, w2_hbm, g_hbm, b_hbm, o_hbm, h_hbm,
            xbuf, obuf, xhead, hbuf, hres, xrem, hrem, orem, xn0_ref, ssq_ref, w1v, w2v,
            bias_ref, sc_ref, dw_ref, g_ref, b_ref,
            xsem, xhsem, osem, hwsem, hrsem, wsem, rsem):
    n = (x_hbm.shape[0] - REM) // TM
    F = w1v.shape[1]
    F0 = SUB0
    NM = REM // MS

    def al(v):
        return pl.multiple_of(v, 16)

    def xcopy(t, s):
        return pltpu.make_async_copy(x_hbm.at[pl.ds(al(REM + t * TM), TM), :], xbuf.at[s], xsem.at[s])

    def xhcopy(t, s):
        return pltpu.make_async_copy(x_hbm.at[pl.ds(al(REM + t * TM), F0), :], xhead.at[s], xhsem.at[s])

    def hwcopy(t, s):
        return pltpu.make_async_copy(hbuf.at[s], h_hbm.at[pl.ds(al(t * SR), SR), :], hwsem.at[s])

    def hrcopy(t, s):
        return pltpu.make_async_copy(h_hbm.at[pl.ds(al(t * SR), SR), :], hbuf.at[s], hrsem.at[s])

    def ocopy(t, s, k):
        lo, hi = _OC[k]
        return pltpu.make_async_copy(obuf.at[s, pl.ds(lo, hi - lo), :],
                                     o_hbm.at[pl.ds(al(REM + t * TM + lo), hi - lo), :], osem.at[s])

    def orcopy(k):
        return pltpu.make_async_copy(orem.at[pl.ds(al(k * MS), MS), :],
                                     o_hbm.at[pl.ds(al(k * MS), MS), :], rsem.at[1])

    w1copy = pltpu.make_async_copy(w1_hbm, w1v, wsem.at[0])
    w2copy = pltpu.make_async_copy(w2_hbm, w2v, wsem.at[1])
    dwcopy = pltpu.make_async_copy(dw_hbm, dw_ref, wsem.at[2])
    gcopy = pltpu.make_async_copy(g_hbm, g_ref, wsem.at[3])
    bcopy = pltpu.make_async_copy(b_hbm, b_ref, wsem.at[4])
    xrcopy = pltpu.make_async_copy(x_hbm.at[pl.ds(0, REM + F0), :], xrem, rsem.at[0])

    def conv_ln(xt, dw):
        y = xt.astype(jnp.float32) * dw
        m = jnp.mean(y, axis=-1, keepdims=True)
        d = y - m
        v = jnp.mean(d * d, axis=-1, keepdims=True)
        return (d * (KS * lax.rsqrt(v + 1e-5))).astype(jnp.bfloat16)

    def expand(xn, put):
        rows = xn.shape[0]
        for c in range(F // NCH):
            a = jnp.dot(xn, w1v[:, c * NCH:(c + 1) * NCH], preferred_element_type=jnp.float32)
            t = jnp.tanh(a * (a * a + A_LIN))
            h = a * (t + 1.0)
            ssq_ref[:, c * NCH:(c + 1) * NCH] += (h * h).reshape(rows // 8, 8, NCH).sum(axis=0)
            put(c, h.astype(jnp.bfloat16))

    dwcopy.start()
    xrcopy.start()
    w1copy.start()
    xcopy(0, 0).start()
    xhcopy(1, 1).start()
    ssq_ref[...] = jnp.zeros_like(ssq_ref)
    dwcopy.wait()
    dw = dw_ref[...].astype(jnp.float32)
    xrcopy.wait()
    xn0_ref[...] = conv_ln(xrem[pl.ds(0, F0), :], dw)
    w1copy.wait()

    def short0(k, carry):
        base = pl.multiple_of(k * MS, MS)
        for (r0, r1) in _ranges(MS, SUB0):
            rows = r1 - r0
            xn = xn0_ref[...] if r0 == 0 else conv_ln(xrem[pl.ds(base + r0, rows), :], dw)

            def put(c, hb):
                hrem[pl.ds(base + r0, rows), c * NCH:(c + 1) * NCH] = hb
            expand(xn, put)
        xn0_ref[...] = conv_ln(xrem[pl.ds(base + MS, F0), :], dw)
        return carry

    lax.fori_loop(0, NM, short0, 0)

    def body0(i, carry):
        slot = i & 1
        nslot = 1 - slot

        @pl.when(i >= 2)
        def _():
            hwcopy(i - 2, slot).wait()

        xcopy(i, slot).wait()

        @pl.when(i + 1 < n)
        def _():
            xhcopy(i + 1, nslot).wait()

        @pl.when(i + 1 < n)
        def _():
            xcopy(i + 1, nslot).start()

        @pl.when(i + 2 < n)
        def _():
            xhcopy(i + 2, slot).start()

        @pl.when(i == 1)
        def _():
            w2copy.start()
            gcopy.start()
            bcopy.start()

        rbase = al(i * RR)
        for (r0, r1) in _ranges(TM, SUB0):
            rows = r1 - r0
            xn = xn0_ref[...] if r0 == 0 else conv_ln(xbuf[slot, pl.ds(r0, rows), :], dw)

            def put(c, hb):
                for res, lo, hi in _pieces(r0, r1):
                    v = hb[lo - r0:hi - r0, :]
                    if res:
                        hres[pl.ds(rbase + (lo - SR), hi - lo), c * NCH:(c + 1) * NCH] = v
                    else:
                        hbuf[slot, pl.ds(lo, hi - lo), c * NCH:(c + 1) * NCH] = v
            expand(xn, put)
            if r0 < SR <= r1:
                @pl.when(i < n - 2)
                def _():
                    hwcopy(i, slot).start()
        xn0_ref[...] = conv_ln(xhead[nslot], dw)
        return carry

    lax.fori_loop(0, n, body0, 0)

    w2copy.wait()
    gcopy.wait()
    bcopy.wait()
    ss = jnp.sum(ssq_ref[...], axis=0, keepdims=True) * (H_SCALE * H_SCALE)
    gx = jnp.sqrt(ss + 1e-6)
    nx = gx / (jnp.mean(gx, axis=-1, keepdims=True) + 1e-6)
    g = g_ref[...].reshape(1, F).astype(jnp.float32)
    sc_ref[...] = jnp.broadcast_to((g * nx + 1.0) * H_SCALE, sc_ref.shape)
    bb = jnp.broadcast_to(b_ref[...].reshape(1, F), (8, F))
    bias_ref[...] = jnp.dot(bb, w2v[...], preferred_element_type=jnp.float32)

    def contract(hb, xres):
        lhs = (hb.astype(jnp.float32) * sc_ref[0:1, :]).astype(jnp.bfloat16)
        acc = jnp.dot(lhs, w2v[...], preferred_element_type=jnp.float32)
        return (acc + bias_ref[0:1, :] + xres.astype(jnp.float32)).astype(jnp.bfloat16)

    def body1(j, carry):
        t = n - 1 - j
        slot = t & 1
        nslot = 1 - slot

        @pl.when(j >= 2)
        def _():
            hrcopy(t, slot).wait()
            xcopy(t, slot).wait()
            for k in range(len(_OC)):
                ocopy(t + 2, slot, k).wait()

        @pl.when(jnp.logical_and(j >= 1, t >= 1))
        def _():
            hrcopy(t - 1, nslot).start()
            xcopy(t - 1, nslot).start()

        rbase = al(t * RR)
        onext = 0
        for (r0, r1) in _ranges(TM, SUB1):
            for res, lo, hi in _pieces(r0, r1):
                if res:
                    hb = hres[pl.ds(rbase + (lo - SR), hi - lo), :]
                else:
                    hb = hbuf[slot, pl.ds(lo, hi - lo), :]
                obuf[slot, pl.ds(lo, hi - lo), :] = contract(hb, xbuf[slot, pl.ds(lo, hi - lo), :])
            while onext < len(_OC) and _OC[onext][1] <= r1:
                ocopy(t, slot, onext).start()
                onext += 1
        return carry

    lax.fori_loop(0, n, body1, 0)

    def short1(k, carry):
        base = pl.multiple_of(k * MS, MS)
        for (r0, r1) in _ranges(MS, SUB1):
            rows = r1 - r0
            orem[pl.ds(base + r0, rows), :] = contract(hrem[pl.ds(base + r0, rows), :],
                                                       xrem[pl.ds(base + r0, rows), :])
        orcopy(k).start()
        return carry

    lax.fori_loop(0, NM, short1, 0)

    for t in (1, 0):
        for k in range(len(_OC)):
            ocopy(t, t % 2, k).wait()
    for k in range(NM):
        orcopy(k).wait()


@jax.jit
def pallas_standalone__modern_conv_block_slak__vision_kernel(x, dw, w1, w2, grn_g, grn_b):
    B, H, W, C = x.shape
    assert B == 1 and dw.shape[:2] == (1, 1)
    N = H * W
    F = w1.shape[1]
    nt = (N - REM) // TM
    assert REM + nt * TM == N and nt >= 3
    bf16 = jnp.bfloat16
    hbm = pl.BlockSpec(memory_space=pl.ANY)
    out, _ = pl.pallas_call(
        _kernel,
        in_specs=[hbm] * 6,
        out_specs=[hbm, hbm],
        out_shape=[
            jax.ShapeDtypeStruct((N, C), x.dtype),
            jax.ShapeDtypeStruct(((nt - 2) * SR, F), bf16),
        ],
        scratch_shapes=[
            pltpu.VMEM((2, TM, C), bf16),
            pltpu.VMEM((2, TM, C), bf16),
            pltpu.VMEM((2, SUB0, C), bf16),
            pltpu.VMEM((2, SR, F), bf16),
            pltpu.VMEM((nt * RR, F), bf16),
            pltpu.VMEM((REM + SUB0, C), bf16),
            pltpu.VMEM((REM, F), bf16),
            pltpu.VMEM((REM, C), bf16),
            pltpu.VMEM((SUB0, C), bf16),
            pltpu.VMEM((8, F), jnp.float32),
            pltpu.VMEM((C, F), bf16),
            pltpu.VMEM((F, C), bf16),
            pltpu.VMEM((8, C), jnp.float32),
            pltpu.VMEM((8, F), jnp.float32),
            pltpu.VMEM((1, C), bf16),
            pltpu.VMEM((F,), bf16),
            pltpu.VMEM((F,), bf16),
            pltpu.SemaphoreType.DMA((2,)),
            pltpu.SemaphoreType.DMA((2,)),
            pltpu.SemaphoreType.DMA((2,)),
            pltpu.SemaphoreType.DMA((2,)),
            pltpu.SemaphoreType.DMA((2,)),
            pltpu.SemaphoreType.DMA((5,)),
            pltpu.SemaphoreType.DMA((2,)),
        ],
        compiler_params=pltpu.CompilerParams(
            vmem_limit_bytes=128 * 1024 * 1024,
            disable_bounds_checks=True,
            disable_semaphore_checks=True),
    )(x.reshape(N, C), dw.reshape(1, C), w1, w2, grn_g, grn_b)
    return out.reshape(B, H, W, C)
```
